```python
import os as _os
_os.environ.setdefault("JAX_PLATFORMS", "cpu")
import jax
import jax.numpy as jnp

def _softmax(x, axis=-1):
    return jax.nn.softmax(x, axis=axis)
def _gelu(x):
    return jax.nn.gelu(x, approximate=True)
def _silu(x):
    return jax.nn.silu(x)
def _sigmoid(x):
    return jax.nn.sigmoid(x)
def _layernorm(x, axis=-1, eps=1e-5):
    m = jnp.mean(x, axis=axis, keepdims=True)
    v = jnp.var(x, axis=axis, keepdims=True)
    return (x - m) / jnp.sqrt(v + eps)
def _scatter_add(tgt, idx, src, axis=0):
    return tgt.at[idx].add(src)
def _segment_sum(src, seg, n):
    return jax.ops.segment_sum(src, seg, n)
class _Rng:
    def __init__(self, key):
        self._k = key
    def _next(self):
        self._k, sub = jax.random.split(self._k)
        return sub
    def normal(self, shape):
        return jax.random.normal(self._next(), shape, dtype=jnp.bfloat16)
    def randint(self, lo, hi, shape):
        return jax.random.randint(self._next(), shape, lo, hi, dtype=jnp.int32)
    def uniform(self, shape, lo=0.0, hi=1.0):
        return jax.random.uniform(self._next(), shape, jnp.bfloat16, lo, hi)
    def permutation(self, n):
        return jax.random.permutation(self._next(), n)


kernel_name = 'gated_mix__linear_kernel_hedgehog__glu_gated_bilinear__prompt'

def setup_inputs():
    _rng = _Rng(jax.random.key(int.from_bytes(__import__("os").urandom(4), "little")))
    _w = (lambda a: (lambda t: t.astype(jnp.bfloat16) if jnp.issubdtype(t.dtype, jnp.floating) else t)(jnp.asarray(a)))
    def _A_setup():
        B, S, D, H = 1, 2048, 512, 32
        Dh = D // H
        return {
            "x": _w((lambda *s: _rng.normal(s) * 0.05)(B, S, D)),
            "wqkv": _w((lambda *s: _rng.normal(s) * 0.8)(D, 3 * D)),
            "w_phi": _w((lambda *s: _rng.normal(s) * 0.8)(H, Dh, Dh) * (Dh ** -0.5)),
            "wo": _w((lambda *s: _rng.normal(s) * 0.05)(D, D)),
        }
    _A_in = _A_setup()

    def _B_setup():
        B, S, D, F = 1, 2048, 512, 1792
        return {
            "x": _w((lambda *s: _rng.normal(s) * 0.05)(B, S, D)),
            "w_gate": _w((lambda *s: _rng.normal(s) * 1.6)(D, F) * (D ** -0.5)),
            "w_up": _w((lambda *s: _rng.normal(s) * 1.6)(D, F) * (D ** -0.5)),
            "w_down": _w((lambda *s: _rng.normal(s) * 1.6)(F, D) * (F ** -0.5)),
        }
    _B_in = _B_setup()

    return {
        "A_x": _A_in["x"],
        "A_wqkv": _A_in["wqkv"],
        "A_w_phi": _A_in["w_phi"],
        "A_wo": _A_in["wo"],
        "B_x": _B_in["x"],
        "B_w_gate": _B_in["w_gate"],
        "B_w_up": _B_in["w_up"],
        "B_w_down": _B_in["w_down"],
        "gate_w": _w((lambda *s: _rng.normal(s) * 0.05)(512) * 16.0),
    }

def reference(A_x, A_wqkv, A_w_phi, A_wo, B_x, B_w_gate, B_w_up, B_w_down, gate_w):
    def _A_ref(x, wqkv, w_phi, wo):
        B, S, D = x.shape
        H = 32; Dh = D // H
        qkv = (lambda x, *d: x.transpose(*d))((x @ wqkv).reshape(B, S, 3, H, Dh), 2, 0, 3, 1, 4)
        q, k, v = qkv[0], qkv[1], qkv[2]
        pq = jnp.einsum("bhsd,hdf->bhsf", q, w_phi)
        pk = jnp.einsum("bhsd,hdf->bhsf", k, w_phi)
        phi_q = jnp.concatenate([_softmax(pq, axis=-1), _softmax(-pq, axis=-1)], axis=-1)
        phi_k = jnp.concatenate([_softmax(pk, axis=-1), _softmax(-pk, axis=-1)], axis=-1)
        kv = jnp.einsum("bhsf,bhsd->bhfd", phi_k, v)
        z  = jnp.einsum("bhsf->bhf", phi_k)
        num = jnp.einsum("bhqf,bhfd->bhqd", phi_q, kv)
        den = jnp.einsum("bhqf,bhf->bhq", phi_q, z)[..., None] + 1e-6
        o = num / den
        return (lambda x, *d: x.transpose(*d))(o, 0, 2, 1, 3).reshape(B, S, D) @ wo

    def _B_ref(x, w_gate, w_up, w_down):
        g = jnp.einsum("bsd,df->bsf", x, w_gate)
        u = jnp.einsum("bsd,df->bsf", x, w_up)
        h = g * u
        return jnp.einsum("bsf,fd->bsd", h, w_down)

    x = A_x
    g = _sigmoid((x * gate_w).sum(-1, keepdims=True))
    a = _A_ref(x, A_wqkv, A_w_phi, A_wo)
    b = _B_ref(x, B_w_gate, B_w_up, B_w_down)
    return g * a + (1 - g) * b
```

```python
import functools
import numpy as np
import jax
import jax.numpy as jnp
from jax import lax
import jax.experimental.pallas as pl
import jax.experimental.pallas.tpu as pltpu

S, D, H, DH, F = 2048, 512, 32, 16, 1792
TS = 512
NT = S // TS
NG = 4
LOG2E = 1.4426950408889634
BF = jnp.bfloat16
F32 = jnp.float32
NT_DIMS = (((1,), (1,)), ((), ()))
FC = 256


def _dot(a, b):
    return jnp.dot(a, b, preferred_element_type=F32)


def _dot_nt(a, b):
    return lax.dot_general(a, b, NT_DIMS, preferred_element_type=F32)


def _all(op, red, t):
    m = red(t, axis=0)
    return op(m, pltpu.roll(m, 4, 0))[None]


def _hedgehog_exp(p):
    e1 = jnp.exp2(p - _all(jnp.maximum, jnp.max, p))
    e2 = jnp.exp2(_all(jnp.minimum, jnp.min, p) - p)
    return e1, e2, _all(jnp.add, jnp.sum, e1), _all(jnp.add, jnp.sum, e2)


def _kernel(x_hbm, wqkv_hbm, wphi_ref, wo_hbm, wg_hbm, wu_hbm, wd_hbm, gw_ref, out_hbm,
            x_v, wqkv_v, wo_v, wg_v, wu_v, wd_v, out_v, wqT_v, wkT_v, kv_v, z_v, kvb_v, h_v,
            xsem, wsem, osem):
    x_cp = [pltpu.make_async_copy(x_hbm.at[pl.ds(i * TS, TS)], x_v.at[pl.ds(i * TS, TS)], xsem.at[i])
            for i in range(NT)]
    wk_cp = pltpu.make_async_copy(wqkv_hbm.at[:, pl.ds(D, D)], wqkv_v.at[1], wsem.at[0])
    wv_cp = pltpu.make_async_copy(wqkv_hbm.at[:, pl.ds(2 * D, D)], wqkv_v.at[2], wsem.at[1])
    wq_cp = pltpu.make_async_copy(wqkv_hbm.at[:, pl.ds(0, D)], wqkv_v.at[0], wsem.at[2])
    wg_cp = pltpu.make_async_copy(wg_hbm, wg_v, wsem.at[3])
    wu_cp = pltpu.make_async_copy(wu_hbm, wu_v, wsem.at[4])
    wd_cp = pltpu.make_async_copy(wd_hbm, wd_v, wsem.at[5])
    wo_cp = pltpu.make_async_copy(wo_hbm, wo_v, wsem.at[6])
    wk_cp.start()
    x_cp[0].start()
    wv_cp.start()
    wq_cp.start()
    for i in range(1, NT):
        x_cp[i].start()
    wg_cp.start()
    wu_cp.start()
    wd_cp.start()
    wo_cp.start()

    row = lax.broadcasted_iota(jnp.int32, (128, 128), 0)
    col = lax.broadcasted_iota(jnp.int32, (128, 128), 1)
    same_head = ((row // 64) * 4 + row % 4) == (col // DH)
    wp = wphi_ref[...].reshape(DH * DH, H)
    srow = lax.broadcasted_iota(jnp.int32, (128, H), 0)
    scol = lax.broadcasted_iota(jnp.int32, (128, H), 1)
    frow = lax.broadcasted_iota(jnp.int32, (128, 256), 0)
    fcol = lax.broadcasted_iota(jnp.int32, (128, 256), 1)
    same_f = ((frow % 64) // 4) == (fcol % DH)
    rrow = lax.broadcasted_iota(jnp.int32, (256, 128), 0)
    rcol = lax.broadcasted_iota(jnp.int32, (256, 128), 1)
    spread_d = jnp.where((rrow // DH) == (rcol % DH), 1.0, 0.0).astype(BF)
    phiT = []
    for g in range(NG):
        sel = jnp.where(scol == (srow // 64) * 4 + srow % 4 + g * 8, 1.0, 0.0).astype(BF)
        t = jnp.where(same_f, _dot_nt(sel, wp), 0.0).astype(BF)
        phiT.append(jnp.where(same_head, _dot(t, spread_d), 0.0).astype(BF))

    def fold(idx, dst):
        for g in range(NG):
            t = _dot_nt(phiT[g], wqkv_v[idx, :, g * 128:(g + 1) * 128])
            dst[g * 128:(g + 1) * 128, :] = (t * LOG2E).astype(BF)

    wk_cp.wait()
    fold(1, wkT_v)
    kv_v[...] = jnp.zeros_like(kv_v)
    z_v[...] = jnp.zeros_like(z_v)
    wv_cp.wait()
    wq_cp.wait()
    fold(0, wqT_v)
    wkT_v[D:2 * D, :] = wqkv_v[2].T

    @pl.loop(0, NT)
    def _(i):
        rows = pl.ds(pl.multiple_of(i * TS, TS), TS)
        pltpu.make_async_copy(x_hbm.at[rows], x_v.at[rows], xsem.at[i]).wait()
        xt = x_v[rows, :]
        pk = _dot_nt(wkT_v[...], xt)
        vT = pk[D:].astype(BF)
        for g in range(8):
            p = pk[g * 64:(g + 1) * 64].reshape(8, 8, TS)
            e1, e2, s1, s2 = _hedgehog_exp(p)
            f1 = (e1 * (1.0 / s1)).reshape(64, TS)
            f2 = (e2 * (1.0 / s2)).reshape(64, TS)
            f12 = jnp.concatenate([f1, f2], axis=0)
            zz = f12[:, 0:128]
            for j in range(1, TS // 128):
                zz = zz + f12[:, j * 128:(j + 1) * 128]
            z_v[g] += zz
            kv_v[g] += _dot_nt(vT[g * 64:(g + 1) * 64], f12.astype(BF))

    sh2 = (lax.broadcasted_iota(jnp.int32, (64, 128), 0) // DH) == (lax.broadcasted_iota(jnp.int32, (64, 128), 1) % 4)
    for g in range(8):
        kvb_v[g] = jnp.where(sh2, kv_v[g], 0.0).astype(BF)
        z_v[g] = jnp.broadcast_to(jnp.sum(z_v[g], axis=1, keepdims=True), (128, 128))

    wg_cp.wait()
    wu_cp.wait()
    wd_cp.wait()
    wo_cp.wait()
    gw = gw_ref[...].reshape(1, D).astype(F32)
    def out_copy(i, n):
        r = pl.ds(pl.multiple_of(i * TS, TS), TS)
        cs = slice(n * 128, (n + 1) * 128)
        return pltpu.make_async_copy(out_v.at[r, cs], out_hbm.at[r, cs], osem.at[i * 4 + n])

    @pl.loop(0, NT)
    def _(i):
        rows = pl.ds(pl.multiple_of(i * TS, TS), TS)
        xt = x_v[rows, :]
        pq = _dot_nt(wqT_v[...], xt)
        os_ = []
        for g in range(8):
            p = pq[g * 64:(g + 1) * 64].reshape(8, 8, TS)
            e1, e2, s1, s2 = _hedgehog_exp(p)
            z = jnp.concatenate([z_v[g]] * (TS // 128), axis=1).reshape(16, 8, TS)
            r1 = 1.0 / s1
            r2 = 1.0 / s2
            d = r1[0] * jnp.sum(e1 * z[:8], axis=0) + r2[0] * jnp.sum(e2 * z[8:], axis=0)
            rd = 1.0 / (d + pltpu.roll(d, 4, 0) + 1e-6)[None]
            f1 = (e1 * (r1 * rd)).reshape(64, TS)
            f2 = (e2 * (r2 * rd)).reshape(64, TS)
            f12 = jnp.concatenate([f1, f2], axis=0).astype(BF)
            os_.append(_dot(kvb_v[g], f12).astype(BF))
        o = jnp.concatenate(os_, axis=0).T
        for c in range(F // FC):
            gg = _dot(xt, wg_v[:, c * FC:(c + 1) * FC])
            uu = _dot(xt, wu_v[:, c * FC:(c + 1) * FC])
            h_v[:, c * FC:(c + 1) * FC] = (gg * uu).astype(BF)
        gate = jax.nn.sigmoid(jnp.sum(xt.astype(F32) * gw, axis=1, keepdims=True))
        for n in range(4):
            cs = slice(n * 128, (n + 1) * 128)
            a = _dot(o, wo_v[:, cs])
            b = _dot(h_v[...], wd_v[:, cs])
            out_v[rows, cs] = (gate * a + (1.0 - gate) * b).astype(BF)
            out_copy(i, n).start()
    for i in range(NT):
        for n in range(4):
            out_copy(i, n).wait()


@jax.jit
def pallas_gated_mix__linear_kernel_hedgehog__glu_gated_bilinear__prompt_kernel(
    A_x, A_wqkv, A_w_phi, A_wo, B_x, B_w_gate, B_w_up, B_w_down, gate_w,
):
    any_spec = pl.BlockSpec(memory_space=pl.ANY)
    vmem_spec = pl.BlockSpec(memory_space=pltpu.VMEM)
    out = pl.pallas_call(
        _kernel,
        in_specs=[any_spec, any_spec, vmem_spec, any_spec, any_spec, any_spec, any_spec, vmem_spec],
        out_specs=any_spec,
        out_shape=jax.ShapeDtypeStruct((S, D), BF),
        scratch_shapes=[
            pltpu.VMEM((S, D), BF), pltpu.VMEM((3, D, D), BF), pltpu.VMEM((D, D), BF),
            pltpu.VMEM((D, F), BF), pltpu.VMEM((D, F), BF), pltpu.VMEM((F, D), BF),
            pltpu.VMEM((S, D), BF), pltpu.VMEM((D, D), BF), pltpu.VMEM((2 * D, D), BF),
            pltpu.VMEM((8, 64, 128), F32), pltpu.VMEM((8, 128, 128), F32), pltpu.VMEM((8, 64, 128), BF),
            pltpu.VMEM((TS, F), BF),
            pltpu.SemaphoreType.DMA((NT,)), pltpu.SemaphoreType.DMA((7,)), pltpu.SemaphoreType.DMA((NT * 4,)),
        ],
        compiler_params=pltpu.CompilerParams(vmem_limit_bytes=100 * 1024 * 1024),
    )(A_x.reshape(S, D), A_wqkv, A_w_phi.transpose(1, 2, 0), A_wo, B_w_gate, B_w_up, B_w_down, gate_w)
    return out.reshape(1, S, D)
```
